```python
import jax
import jax.numpy as jnp

def _softmax(x, axis=-1):
    return jax.nn.softmax(x, axis=axis)

def _gelu(x):
    return jax.nn.gelu(x, approximate=True)

def _silu(x):
    return jax.nn.silu(x)

def _sigmoid(x):
    return jax.nn.sigmoid(x)

def _layernorm(x, axis=-1, eps=1e-05):
    m = jnp.mean(x, axis=axis, keepdims=True)
    v = jnp.var(x, axis=axis, keepdims=True)
    return (x - m) / jnp.sqrt(v + eps)

def _scatter_add(tgt, idx, src, axis=0):
    return tgt.at[idx].add(src)

def _segment_sum(src, seg, n):
    return jax.ops.segment_sum(src, seg, n)

class _Rng:

    def __init__(self, key):
        self._k = key

    def _next(self):
        self._k, sub = jax.random.split(self._k)
        return sub

    def normal(self, shape):
        return jax.random.normal(self._next(), shape, dtype=jnp.bfloat16)

    def randint(self, lo, hi, shape):
        return jax.random.randint(self._next(), shape, lo, hi, dtype=jnp.int32)

    def uniform(self, shape, lo=0.0, hi=1.0):
        return jax.random.uniform(self._next(), shape, jnp.bfloat16, lo, hi)

    def permutation(self, n):
        return jax.random.permutation(self._next(), n)
kernel_name = 'adaLN_cond__ssm_conv_h3__mixer_s_mlp__prompt'

def setup_inputs():
    _rng = _Rng(jax.random.key(int.from_bytes(__import__("os").urandom(4), "little")))
    _w = lambda a: (lambda t: t.astype(jnp.bfloat16) if jnp.issubdtype(t.dtype, jnp.floating) else t)(jnp.asarray(a))

    def _A_setup():
        B, S, D = (1, 2048, 640)
        ks = 4
        return {'q': _w((lambda *s: _rng.normal(s) * 0.05)(B, S, D)), 'k': _w((lambda *s: _rng.normal(s) * 0.05)(B, S, D)), 'v': _w((lambda *s: _rng.normal(s) * 0.05)(B, S, D)), 'shift_k': _w((lambda *s: _rng.normal(s) * 0.05)(D, ks) * 0.5), 'ssm_k': _w((lambda *s: _rng.normal(s) * 0.05)(D, S) * (1.0 / S ** 0.5)), 'ssm_D': _w((lambda *s: _rng.normal(s) * 0.05)(D))}
    _A_in = _A_setup()

    def _B_setup():
        B, S, D, F = (1, 2048, 640, 1728)
        return {'x': _w((lambda *s: _rng.normal(s) * 0.05)(B, S, D)), 'w1': _w((lambda *s: _rng.normal(s) * 0.05)(D, D) * D ** (-0.5)), 'w2': _w((lambda *s: _rng.normal(s) * 0.05)(D, D) * D ** (-0.5)), 'w3': _w((lambda *s: _rng.normal(s) * 0.05)(D, F) * D ** (-0.5)), 'w4': _w((lambda *s: _rng.normal(s) * 0.05)(F, D) * F ** (-0.5))}
    _B_in = _B_setup()
    return {'A_q': _A_in['q'], 'A_k': _A_in['k'], 'A_v': _A_in['v'], 'A_shift_k': _A_in['shift_k'], 'A_ssm_k': _A_in['ssm_k'], 'A_ssm_D': _A_in['ssm_D'], 'B_x': _B_in['x'], 'B_w1': _B_in['w1'], 'B_w2': _B_in['w2'], 'B_w3': _B_in['w3'], 'B_w4': _B_in['w4'], 'c': _w((lambda *s: _rng.normal(s) * 0.05)(1, 640)), 'w_mod': _w((lambda *s: _rng.normal(s) * 0.05)(640, 6 * 640) * 640 ** (-0.5))}

def reference(A_q, A_k, A_v, A_shift_k, A_ssm_k, A_ssm_D, B_x, B_w1, B_w2, B_w3, B_w4, c, w_mod):

    def _A_ref(q, k, v, shift_k, ssm_k, ssm_D):
        B, S, D = q.shape
        ks = shift_k.shape[-1]
        k_pad = jnp.pad(k, ((0, 0), (ks - 1, 0), (0, 0)))
        k_shift = jnp.zeros_like(k)
        for t in range(ks):
            k_shift = k_shift + k_pad[:, t:t + S, :] * shift_k[:, ks - 1 - t][None, None, :]
        kv = k_shift * v
        L = 2 * S
        kv_pad = jnp.pad(kv, ((0, 0), (0, S), (0, 0)))
        kf_pad = jnp.pad(ssm_k, ((0, 0), (0, S)))
        kv_f = (lambda x, axes=(-2, -1): jnp.fft.rfft2(x.astype(jnp.float32), axes=axes))(kv_pad[:, None, :, :], axes=(1, 2))
        kf_f = (lambda x, axes=(-2, -1): jnp.fft.rfft2(x.astype(jnp.float32), axes=axes))(kf_pad[:, None, :], axes=(1, 2))
        kf_f = (lambda x, *d: x.transpose(*d))(kf_f, 1, 2, 0)
        y_f = kv_f * kf_f[None, :, :, :]
        y = (lambda x, s, axes=(-2, -1): jnp.fft.irfft2(x, s=s, axes=axes).astype(jnp.bfloat16))(y_f, (1, L), axes=(1, 2))[:, 0, :S, :]
        y = y + kv * ssm_D[None, None, :]
        return q * y

    def _B_ref(x, w1, w2, w3, w4):
        B, S, D = x.shape
        h = _gelu(_layernorm(x, axis=-1) @ w1)
        c = D // 4
        g0 = jnp.pad(h[:, :, 0 * c:1 * c], ((0, 0), (1, 0), (0, 0)))[:, :S, :]
        g1 = jnp.pad(h[:, :, 1 * c:2 * c], ((0, 0), (0, 1), (0, 0)))[:, 1:, :]
        g2 = jnp.pad(h[:, :, 2 * c:3 * c], ((0, 0), (2, 0), (0, 0)))[:, :S, :]
        g3 = jnp.pad(h[:, :, 3 * c:], ((0, 0), (0, 2), (0, 0)))[:, 2:, :]
        hs = jnp.concatenate([g0, g1, g2, g3], axis=-1) @ w2
        x1 = x + hs
        h2 = _gelu(_layernorm(x1, axis=-1) @ w3) @ w4
        return x1 + h2
    x = A_q
    mod = (_silu(c) @ w_mod).reshape(c.shape[0], 6, 1, -1)
    sa, ca, ga, sb, cb, gb = (mod[:, 0].copy(), mod[:, 1].copy(), mod[:, 2].copy(), mod[:, 3].copy(), mod[:, 4].copy(), mod[:, 5].copy())
    h = _layernorm(x, axis=-1) * (1 + ca) + sa
    x = x + ga * _A_ref(h, A_k, A_v, A_shift_k, A_ssm_k, A_ssm_D)
    h = _layernorm(x, axis=-1) * (1 + cb) + sb
    x = x + gb * _B_ref(h, B_w1, B_w2, B_w3, B_w4)
    return x
```

```python
import numpy as np
import jax
import jax.numpy as jnp
from jax import lax
import jax.experimental.pallas as pl
import jax.experimental.pallas.tpu as pltpu

S, D, FF = 2048, 640, 1728
BLK = 128
NB = S // BLK
R = 256
NR = S // R
EPS = 1e-5
F32, BF16 = jnp.float32, jnp.bfloat16


def _dft_matrix():
    f = np.arange(BLK)[:, None]
    n = np.arange(BLK)[None, :]
    ang = np.pi * ((2 * f + 1) * n % (4 * BLK)) / (2 * BLK)
    return np.concatenate([np.cos(ang), -np.sin(ang)], axis=0).astype(np.float32)


def _ln(x):
    m = jnp.mean(x, axis=-1, keepdims=True)
    xc = x - m
    v = jnp.mean(xc * xc, axis=-1, keepdims=True)
    return xc * lax.rsqrt(v + EPS)


_C1 = float(np.sqrt(2.0 / np.pi))
_C2 = float(np.sqrt(2.0 / np.pi) * 0.044715)


def _gelu(x):
    t = jnp.tanh(x * (_C1 + _C2 * (x * x)))
    hx = 0.5 * x
    return hx + hx * t


def _mm(a, b):
    return jnp.dot(a, b, preferred_element_type=F32)


def _mmt(a, b):
    return lax.dot_general(a, b, (((1,), (1,)), ((), ())), preferred_element_type=F32)


def _kernel(q_hbm, k_hbm, v_hbm, ssm_hbm, w1_hbm, w2_hbm, w3_hbm, w4_hbm, wm_hbm,
            sh_ref, sd_ref, c_ref, f_ref, fi_ref, o_hbm,
            q_v, k_v, v_v, ssm_v, w1_v, w2_v, w3_v, w4_v, wm_v,
            kv_v, u_v, g_v, z_v, x2_v, hb_v, ge_v, o_v,
            sem_k, sem_v, sem_s, sem_w, sem_o):
    def k_cp(i):
        return pltpu.make_async_copy(k_hbm.at[pl.ds(i * BLK, BLK)],
                                     k_v.at[pl.ds(16 + i * BLK, BLK)], sem_k.at[i])

    def v_cp(i):
        return pltpu.make_async_copy(v_hbm.at[pl.ds(i * BLK, BLK)],
                                     v_v.at[pl.ds(i * BLK, BLK)], sem_v.at[i])

    def s_cp(i):
        return pltpu.make_async_copy(ssm_hbm.at[:, pl.ds(i * BLK, BLK)], ssm_v.at[i], sem_s.at[i])

    def o_cp(r):
        return pltpu.make_async_copy(o_v.at[pl.ds(r * R, R)], o_hbm.at[pl.ds(r * R, R)], sem_o.at[r])

    for i in range(NB):
        s_cp(i).start()
        k_cp(i).start()
        v_cp(i).start()
    wcp = [pltpu.make_async_copy(a, b, sem_w.at[n]) for n, (a, b) in enumerate(
        [(wm_hbm, wm_v), (q_hbm, q_v), (w1_hbm, w1_v), (w2_hbm, w2_v), (w3_hbm, w3_v), (w4_hbm, w4_v)])]
    for cp in wcp:
        cp.start()

    k_v[0:16, :] = jnp.zeros((16, D), BF16)
    ge_v[0:8, :] = jnp.zeros((8, D), F32)
    ge_v[S + 8:S + 16, :] = jnp.zeros((8, D), F32)
    sh = sh_ref[...].astype(F32)
    sgn = jnp.where(lax.broadcasted_iota(jnp.int32, (BLK, D), 0) % 2 == 0, 1.0, -1.0).astype(F32)

    g_v[NB] = jnp.zeros((2 * BLK, D), F32)

    def fwd(i, _):
        k_cp(i).wait()
        v_cp(i).wait()
        s_cp(i).wait()
        r0 = pl.multiple_of(i * BLK, BLK)
        kk = k_v[pl.ds(r0, BLK + 16), :].astype(F32)
        ks = kk[16:16 + BLK] * sh[0:1]
        for j in range(1, 4):
            ks = ks + kk[16 - j:16 - j + BLK] * sh[j:j + 1]
        kv = (ks * v_v[pl.ds(r0, BLK), :].astype(F32)).astype(BF16)
        kv_v[pl.ds(r0, BLK), :] = kv
        f = f_ref[...]
        u_v[i] = _mm(f, kv)
        h = lax.dot_general(f, ssm_v[i], (((1,), (1,)), ((), ())), preferred_element_type=F32)
        hp = g_v[NB]
        g_v[i, 0:BLK, :] = h[0:BLK] - sgn * hp[BLK:]
        g_v[i, BLK:, :] = h[BLK:] + sgn * hp[0:BLK]
        g_v[NB] = h
        return 0

    lax.fori_loop(0, NB, fwd, 0)

    def freq(p, _):
        fr = pl.multiple_of((p % 8) * 16, 16)
        cl = pl.multiple_of((p // 8) * 128, 128)
        re = (pl.ds(fr, 16), pl.ds(cl, 128))
        im = (pl.ds(fr + BLK, 16), pl.ds(cl, 128))
        for i in range(NB):
            zr = zi = None
            for m in range(i + 1):
                gr, gi = g_v[(m, *re)], g_v[(m, *im)]
                ur, ui = u_v[(i - m, *re)], u_v[(i - m, *im)]
                a = gr * ur - gi * ui
                b = gr * ui + gi * ur
                zr = a if zr is None else zr + a
                zi = b if zi is None else zi + b
            z_v[(i, *re)] = zr.astype(BF16)
            z_v[(i, *im)] = zi.astype(BF16)
        return 0

    lax.fori_loop(0, 40, freq, 0)

    wcp[0].wait()
    cc = c_ref[...].astype(F32)
    sc = (cc * jax.nn.sigmoid(cc)).astype(BF16)
    mod = _mm(jnp.broadcast_to(sc, (8, D)), wm_v[...])[0:1]
    sa, ca, ga, sb, cb, gb = [mod[:, n * D:(n + 1) * D] for n in range(6)]
    ca1, cb1 = 1.0 + ca, 1.0 + cb
    sd = sd_ref[...].astype(F32).reshape(1, D)
    wcp[1].wait()
    wcp[2].wait()

    def mid(r, _):
        r0 = pl.multiple_of(r * R, R)
        fi = fi_ref[...]
        y = jnp.concatenate([_mm(fi, z_v[r * (R // BLK) + b]) for b in range(R // BLK)], axis=0)
        y = y + kv_v[pl.ds(r0, R), :].astype(F32) * sd
        x = q_v[pl.ds(r0, R), :].astype(F32)
        h = _ln(x) * ca1 + sa
        x2 = x + ga * (h * y)
        hb = _ln(x2) * cb1 + sb
        x2_v[pl.ds(r0, R), :] = x2
        hb_v[pl.ds(r0, R), :] = hb
        ge_v[pl.ds(r0 + 8, R), :] = _gelu(_mm(_ln(hb).astype(BF16), w1_v[...]))
        return 0

    lax.fori_loop(0, NR, mid, 0)
    wcp[3].wait()
    wcp[4].wait()
    wcp[5].wait()
    lane = lax.broadcasted_iota(jnp.int32, (R, 128), 1)

    def tail(r, _):
        r0 = pl.multiple_of(r * R, R)
        ge = ge_v[pl.ds(r0, R + 16), :]

        def sft(t, d):
            return ge[8 - d:8 - d + R, t * 128:(t + 1) * 128]

        gs = jnp.concatenate([
            sft(0, 1),
            jnp.where(lane < 32, sft(1, 1), sft(1, -1)),
            jnp.where(lane < 64, sft(2, -1), sft(2, 2)),
            jnp.where(lane < 96, sft(3, 2), sft(3, -2)),
            sft(4, -2)], axis=1).astype(BF16)
        x1 = hb_v[pl.ds(r0, R), :] + _mm(gs, w2_v[...])
        h2 = _gelu(_mmt(_ln(x1).astype(BF16), w3_v[...])).astype(BF16)
        out = x2_v[pl.ds(r0, R), :] + gb * (x1 + _mm(h2, w4_v[...]))
        o_v[pl.ds(r0, R), :] = out.astype(BF16)
        o_cp(r).start()
        return 0

    lax.fori_loop(0, NR, tail, 0)
    for r in range(NR):
        o_cp(r).wait()


@jax.jit
def pallas_adaLN_cond__ssm_conv_h3__mixer_s_mlp__prompt_kernel(
    A_q: jax.Array,
    A_k: jax.Array,
    A_v: jax.Array,
    A_shift_k: jax.Array,
    A_ssm_k: jax.Array,
    A_ssm_D: jax.Array,
    B_x: jax.Array,
    B_w1: jax.Array,
    B_w2: jax.Array,
    B_w3: jax.Array,
    B_w4: jax.Array,
    c: jax.Array,
    w_mod: jax.Array,
):
    del B_x
    f = _dft_matrix()
    f_c = jnp.asarray(f, dtype=BF16)
    fi_c = jnp.asarray(f.T / BLK, dtype=BF16)
    hbm = pl.BlockSpec(memory_space=pl.ANY)
    vm = pl.BlockSpec(memory_space=pltpu.VMEM)
    out = pl.pallas_call(
        _kernel,
        in_specs=[hbm] * 9 + [vm] * 5,
        out_specs=hbm,
        out_shape=jax.ShapeDtypeStruct((S, D), BF16),
        scratch_shapes=[
            pltpu.VMEM((S, D), BF16), pltpu.VMEM((S + 16, D), BF16), pltpu.VMEM((S, D), BF16),
            pltpu.VMEM((NB, D, BLK), BF16),
            pltpu.VMEM((D, D), BF16), pltpu.VMEM((D, D), BF16),
            pltpu.VMEM((FF, D), BF16), pltpu.VMEM((FF, D), BF16), pltpu.VMEM((D, 6 * D), BF16),
            pltpu.VMEM((S, D), BF16),
            pltpu.VMEM((NB, 2 * BLK, D), F32), pltpu.VMEM((NB + 1, 2 * BLK, D), F32),
            pltpu.VMEM((NB, 2 * BLK, D), BF16),
            pltpu.VMEM((S, D), F32), pltpu.VMEM((S, D), F32), pltpu.VMEM((S + 16, D), F32),
            pltpu.VMEM((S, D), BF16),
            pltpu.SemaphoreType.DMA((NB,)), pltpu.SemaphoreType.DMA((NB,)),
            pltpu.SemaphoreType.DMA((NB,)), pltpu.SemaphoreType.DMA((6,)),
            pltpu.SemaphoreType.DMA((NR,)),
        ],
        compiler_params=pltpu.CompilerParams(vmem_limit_bytes=110 * 1024 * 1024),
    )(A_q.reshape(S, D), A_k.reshape(S, D), A_v.reshape(S, D), A_ssm_k, B_w1, B_w2, B_w3.T, B_w4,
      w_mod, A_shift_k.T, A_ssm_D, c, f_c, fi_c)
    return out.reshape(1, S, D)
```

```python
import functools

import numpy as np
import jax
import jax.numpy as jnp
from jax import lax
import jax.experimental.pallas as pl
import jax.experimental.pallas.tpu as pltpu

S, D, FF = 2048, 640, 1728
BLK = 128
NB = S // BLK
R = 256
NR = S // R
FC = 512
LEAD = 5
FLEAD = 4
EPS = 1e-5
F32, BF16 = jnp.float32, jnp.bfloat16


def _dft_matrix():
    f = np.arange(BLK)[:, None]
    n = np.arange(BLK)[None, :]
    ang = np.pi * ((2 * f + 1) * n % (4 * BLK)) / (2 * BLK)
    return np.concatenate([np.cos(ang), -np.sin(ang)], axis=0).astype(np.float32)


def _ln(x):
    m = jnp.mean(x, axis=-1, keepdims=True)
    xc = x - m
    v = jnp.mean(xc * xc, axis=-1, keepdims=True)
    return xc * lax.rsqrt(v + EPS)


_C1 = float(np.sqrt(2.0 / np.pi))
_C2 = float(np.sqrt(2.0 / np.pi) * 0.044715)


def _gelu(x):
    t = jnp.tanh(x * (_C1 + _C2 * (x * x)))
    hx = 0.5 * x
    return hx + hx * t


def _mm(a, b):
    return jnp.dot(a, b, preferred_element_type=F32)


def _mmt(a, b):
    return lax.dot_general(a, b, (((1,), (1,)), ((), ())), preferred_element_type=F32)


def _kernel(q_hbm, k_hbm, v_hbm, ssm_hbm, w1_hbm, w2_hbm, w3_hbm, w4_hbm, wm_hbm,
            sh_ref, sd_ref, c_ref, f_ref, fi_ref, o_hbm,
            q_v, k_v, v_v, ssm_v, w1_v, w2_v, w3_v, w4_v, wm_v,
            kv_v, u_v, g_v, y_v, z_v, x2_v, hb_v, ge_v, o_v,
            sem_k, sem_v, sem_s, sem_w, sem_q, sem_o):
    def k_cp(i):
        return pltpu.make_async_copy(k_hbm.at[pl.ds(i * BLK, BLK)],
                                     k_v.at[pl.ds(16 + i * BLK, BLK)], sem_k.at[i])

    def v_cp(i):
        return pltpu.make_async_copy(v_hbm.at[pl.ds(i * BLK, BLK)],
                                     v_v.at[pl.ds(i * BLK, BLK)], sem_v.at[i])

    def s_cp(i):
        return pltpu.make_async_copy(ssm_hbm.at[:, pl.ds(i * BLK, BLK)], ssm_v.at[i], sem_s.at[i])

    def o_cp(r):
        return pltpu.make_async_copy(o_v.at[pl.ds(r * R, R)], o_hbm.at[pl.ds(r * R, R)], sem_o.at[r])

    def q_cp(r):
        return pltpu.make_async_copy(q_hbm.at[pl.ds(r * R, R)], q_v.at[pl.ds(r * R, R)], sem_q.at[r])

    def conv_in(r, start):
        for i in (2 * r, 2 * r + 1):
            for cp in (s_cp(i), k_cp(i), v_cp(i)):
                cp.start() if start else cp.wait()

    wcp = [pltpu.make_async_copy(a, b, sem_w.at[n]) for n, (a, b) in enumerate(
        [(wm_hbm, wm_v), (w1_hbm, w1_v), (w2_hbm, w2_v), (w3_hbm, w3_v), (w4_hbm, w4_v)])]
    for r in range(LEAD):
        conv_in(r, True)
    for cp in (wcp[0], q_cp(0), wcp[1], q_cp(1), wcp[2], wcp[3], wcp[4]):
        cp.start()
    for r in range(NR):
        if r + LEAD < NR:
            conv_in(r + LEAD, True)
        if r + 2 < NR:
            q_cp(r + 2).start()

    k_v[0:16, :] = jnp.zeros((16, D), BF16)
    ge_v[0:8, :] = jnp.zeros((8, D), F32)
    ge_v[S + 8:S + 16, :] = jnp.zeros((8, D), F32)
    sh = sh_ref[...].astype(F32)
    sgn = jnp.where(lax.broadcasted_iota(jnp.int32, (16, 128), 0) % 2 == 0, 1.0, -1.0).astype(F32)
    lane = lax.broadcasted_iota(jnp.int32, (R, 128), 1)
    P = {}

    def fwd_items(r):
        def one(i, t):
            cs = slice(t * 128, (t + 1) * 128)
            r0 = i * BLK
            kk = k_v[r0:r0 + BLK + 16, cs].astype(F32)
            ks = kk[16:16 + BLK] * sh[0:1, cs]
            for j in range(1, 4):
                ks = ks + kk[16 - j:16 - j + BLK] * sh[j:j + 1, cs]
            kv = (ks * v_v[r0:r0 + BLK, cs].astype(F32)).astype(BF16)
            kv_v[r0:r0 + BLK, cs] = kv
            f = f_ref[...]
            u_v[i, :, cs] = _mm(f, kv)
            g_v[i, :, cs] = _mmt(f, ssm_v[i, cs, :])
        return [functools.partial(one, 2 * r + b, t) for b in range(2) for t in range(5)]

    def freq_items(r):
        def one(p):
            fr, cl = (p % 8) * 16, (p // 8) * 128
            re = (slice(fr, fr + 16), slice(cl, cl + 128))
            im = (slice(fr + BLK, fr + BLK + 16), slice(cl, cl + 128))
            pr = pi = None
            if r > 0:
                pr, pi = y_v[re], y_v[im]
            for i in (2 * r, 2 * r + 1):
                zr = zi = None
                for m in range(i + 1):
                    gr, gi = g_v[(m, *re)], g_v[(m, *im)]
                    ur, ui = u_v[(i - m, *re)], u_v[(i - m, *im)]
                    a = gr * ur - gi * ui
                    b = gr * ui + gi * ur
                    zr = a if zr is None else zr + a
                    zi = b if zi is None else zi + b
                if pr is None:
                    z_v[(i, *re)] = zr.astype(BF16)
                    z_v[(i, *im)] = zi.astype(BF16)
                else:
                    z_v[(i, *re)] = (zr - sgn * pi).astype(BF16)
                    z_v[(i, *im)] = (zi + sgn * pr).astype(BF16)
                pr, pi = zr, zi
            if r < NR - 1:
                y_v[re] = pr
                y_v[im] = pi
        return [functools.partial(one, p) for p in range(40)]

    def mid_items(r):
        def one():
            r0 = r * R
            rs = slice(r0, r0 + R)
            y = jnp.concatenate([_mm(fi_ref[...], z_v[2 * r + b]) for b in range(2)], axis=0)
            y = y + kv_v[rs, :].astype(F32) * P['sd']
            x = q_v[rs, :].astype(F32)
            h = _ln(x) * P['ca1'] + P['sa']
            x2 = x + P['ga'] * (h * y)
            hb = _ln(x2) * P['cb1'] + P['sb']
            x2_v[rs, :] = x2
            hb_v[rs, :] = hb
            ge_v[r0 + 8:r0 + 8 + R, :] = _gelu(_mm(_ln(hb).astype(BF16), w1_v[...]))
        return [one]

    def tail_items(r):
        r0 = r * R
        st = {}

        def head():
            ge = ge_v[r0:r0 + R + 16, :]

            def sft(t, d):
                return ge[8 - d:8 - d + R, t * 128:(t + 1) * 128]

            gs = jnp.concatenate([
                sft(0, 1),
                jnp.where(lane < 32, sft(1, 1), sft(1, -1)),
                jnp.where(lane < 64, sft(2, -1), sft(2, 2)),
                jnp.where(lane < 96, sft(3, 2), sft(3, -2)),
                sft(4, -2)], axis=1).astype(BF16)
            x1 = hb_v[r0:r0 + R, :] + _mm(gs, w2_v[...])
            st['acc'] = x1
            st['l'] = _ln(x1).astype(BF16)

        def ffn(c0, c1):
            h2 = _gelu(_mmt(st['l'], w3_v[c0:c1, :])).astype(BF16)
            st['acc'] = st['acc'] + _mm(h2, w4_v[c0:c1, :])

        def fin():
            o_v[r0:r0 + R, :] = (x2_v[r0:r0 + R, :] + P['gb'] * st['acc']).astype(BF16)
            o_cp(r).start()
        return [head] + [functools.partial(ffn, c, min(c + FC, FF)) for c in range(0, FF, FC)] + [fin]

    def run(*lists):
        lists = [l for l in lists if l]
        order = sorted(((k + 0.5) / len(l), n, k) for n, l in enumerate(lists) for k in range(len(l)))
        order = sorted(order, key=lambda t: t[0] if t[1] != 1 else 0.15)
        for _, n, k in order:
            lists[n][k]()

    def ok(r):
        return 0 <= r < NR

    T = [tail_items(r) for r in range(NR)]
    for s in range(-LEAD, NR + 2):
        if ok(s + LEAD):
            conv_in(s + LEAD, False)
        if s == 0:
            q_cp(s).wait()
        if s == 0:
            wcp[0].wait()
            cc = c_ref[...].astype(F32)
            sc = (cc * jax.nn.sigmoid(cc)).astype(BF16)
            mod = _mm(jnp.broadcast_to(sc, (8, D)), wm_v[...])[0:1]
            sa, ca, ga, sb, cb, gb = [mod[:, n * D:(n + 1) * D] for n in range(6)]
            P.update(sa=sa, ga=ga, sb=sb, gb=gb, ca1=1.0 + ca, cb1=1.0 + cb,
                     sd=sd_ref[...].astype(F32).reshape(1, D))
            wcp[1].wait()
        if s == 2:
            wcp[2].wait()
            wcp[3].wait()
            wcp[4].wait()
        run(T[s - 2] if ok(s - 2) else [],
            mid_items(s) if ok(s) else [],
            freq_items(s + FLEAD) if ok(s + FLEAD) else [],
            fwd_items(s + LEAD) if ok(s + LEAD) else [],
            [q_cp(s + 1).wait] if ok(s) and ok(s + 1) else [])
    for r in range(NR):
        o_cp(r).wait()


@jax.jit
def pallas_adaLN_cond__ssm_conv_h3__mixer_s_mlp__prompt_kernel(
    A_q: jax.Array,
    A_k: jax.Array,
    A_v: jax.Array,
    A_shift_k: jax.Array,
    A_ssm_k: jax.Array,
    A_ssm_D: jax.Array,
    B_x: jax.Array,
    B_w1: jax.Array,
    B_w2: jax.Array,
    B_w3: jax.Array,
    B_w4: jax.Array,
    c: jax.Array,
    w_mod: jax.Array,
):
    del B_x
    f = _dft_matrix()
    f_c = jnp.asarray(f, dtype=BF16)
    fi_c = jnp.asarray(f.T / BLK, dtype=BF16)
    hbm = pl.BlockSpec(memory_space=pl.ANY)
    vm = pl.BlockSpec(memory_space=pltpu.VMEM)
    out = pl.pallas_call(
        _kernel,
        in_specs=[hbm] * 9 + [vm] * 5,
        out_specs=hbm,
        out_shape=jax.ShapeDtypeStruct((S, D), BF16),
        scratch_shapes=[
            pltpu.VMEM((S, D), BF16), pltpu.VMEM((S + 16, D), BF16), pltpu.VMEM((S, D), BF16),
            pltpu.VMEM((NB, D, BLK), BF16),
            pltpu.VMEM((D, D), BF16), pltpu.VMEM((D, D), BF16),
            pltpu.VMEM((FF, D), BF16), pltpu.VMEM((FF, D), BF16), pltpu.VMEM((D, 6 * D), BF16),
            pltpu.VMEM((S, D), BF16),
            pltpu.VMEM((NB, 2 * BLK, D), F32), pltpu.VMEM((NB, 2 * BLK, D), F32),
            pltpu.VMEM((2 * BLK, D), F32),
            pltpu.VMEM((NB, 2 * BLK, D), BF16),
            pltpu.VMEM((S, D), F32), pltpu.VMEM((S, D), F32), pltpu.VMEM((S + 16, D), F32),
            pltpu.VMEM((S, D), BF16),
            pltpu.SemaphoreType.DMA((NB,)), pltpu.SemaphoreType.DMA((NB,)),
            pltpu.SemaphoreType.DMA((NB,)), pltpu.SemaphoreType.DMA((5,)),
            pltpu.SemaphoreType.DMA((NR,)),
            pltpu.SemaphoreType.DMA((NR,)),
        ],
        compiler_params=pltpu.CompilerParams(vmem_limit_bytes=110 * 1024 * 1024),
    )(A_q.reshape(S, D), A_k.reshape(S, D), A_v.reshape(S, D), A_ssm_k, B_w1, B_w2, B_w3.T, B_w4,
      w_mod, A_shift_k.T, A_ssm_D, c, f_c, fi_c)
    return out.reshape(1, S, D)
```
